```python
import os as _os
_os.environ.setdefault("JAX_PLATFORMS", "cpu")
import jax
import jax.numpy as jnp

def _softmax(x, axis=-1):
    return jax.nn.softmax(x, axis=axis)
def _gelu(x):
    return jax.nn.gelu(x, approximate=True)
def _silu(x):
    return jax.nn.silu(x)
def _sigmoid(x):
    return jax.nn.sigmoid(x)
def _layernorm(x, axis=-1, eps=1e-5):
    m = jnp.mean(x, axis=axis, keepdims=True)
    v = jnp.var(x, axis=axis, keepdims=True)
    return (x - m) / jnp.sqrt(v + eps)
def _scatter_add(tgt, idx, src, axis=0):
    return tgt.at[idx].add(src)
def _segment_sum(src, seg, n):
    return jax.ops.segment_sum(src, seg, n)
class _Rng:
    def __init__(self, key):
        self._k = key
    def _next(self):
        self._k, sub = jax.random.split(self._k)
        return sub
    def normal(self, shape):
        return jax.random.normal(self._next(), shape, dtype=jnp.bfloat16)
    def randint(self, lo, hi, shape):
        return jax.random.randint(self._next(), shape, lo, hi, dtype=jnp.int32)
    def uniform(self, shape, lo=0.0, hi=1.0):
        return jax.random.uniform(self._next(), shape, jnp.bfloat16, lo, hi)
    def permutation(self, n):
        return jax.random.permutation(self._next(), n)


kernel_name = 'parallel_sum__linear_kernel_hedgehog__dense_activation_gelu__prompt'

def setup_inputs():
    _rng = _Rng(jax.random.key(int.from_bytes(__import__("os").urandom(4), "little")))
    _w = (lambda a: (lambda t: t.astype(jnp.bfloat16) if jnp.issubdtype(t.dtype, jnp.floating) else t)(jnp.asarray(a)))
    def _A_setup():
        B, S, D, H = 1, 2048, 448, 16
        Dh = D // H
        return {
            "x": _w((lambda *s: _rng.normal(s) * 0.05)(B, S, D)),
            "wqkv": _w((lambda *s: _rng.normal(s) * 0.2)(D, 3 * D)),
            "w_phi": _w((lambda *s: _rng.normal(s) * 0.2)(H, Dh, Dh) * (Dh ** -0.5)),
            "wo": _w((lambda *s: _rng.normal(s) * 0.05)(D, D)),
        }
    _A_in = _A_setup()

    def _B_setup():
        B, S, D, F = 1, 2048, 448, 1792
        return {
            "x": _w((lambda *s: _rng.normal(s) * 0.05)(B, S, D)),
            "w1": _w((lambda *s: _rng.normal(s) * 0.2)(D, F) * (D ** -0.5)),
            "b1": _w((lambda *s: _rng.normal(s) * 0.2)(F) * 0.01),
            "w2": _w((lambda *s: _rng.normal(s) * 0.2)(F, D) * (F ** -0.5)),
            "b2": _w((lambda *s: _rng.normal(s) * 0.05)(D) * 0.01),
        }
    _B_in = _B_setup()

    return {
        "A_x": _A_in["x"],
        "A_wqkv": _A_in["wqkv"],
        "A_w_phi": _A_in["w_phi"],
        "A_wo": _A_in["wo"],
        "B_x": _B_in["x"],
        "B_w1": _B_in["w1"],
        "B_b1": _B_in["b1"],
        "B_w2": _B_in["w2"],
        "B_b2": _B_in["b2"],
    }

def reference(A_x, A_wqkv, A_w_phi, A_wo, B_x, B_w1, B_b1, B_w2, B_b2):
    def _A_ref(x, wqkv, w_phi, wo):
        B, S, D = x.shape
        H = 16; Dh = D // H
        qkv = (lambda x, *d: x.transpose(*d))((x @ wqkv).reshape(B, S, 3, H, Dh), 2, 0, 3, 1, 4)
        q, k, v = qkv[0], qkv[1], qkv[2]
        pq = jnp.einsum("bhsd,hdf->bhsf", q, w_phi)
        pk = jnp.einsum("bhsd,hdf->bhsf", k, w_phi)
        phi_q = jnp.concatenate([_softmax(pq, axis=-1), _softmax(-pq, axis=-1)], axis=-1)
        phi_k = jnp.concatenate([_softmax(pk, axis=-1), _softmax(-pk, axis=-1)], axis=-1)
        kv = jnp.einsum("bhsf,bhsd->bhfd", phi_k, v)
        z  = jnp.einsum("bhsf->bhf", phi_k)
        num = jnp.einsum("bhqf,bhfd->bhqd", phi_q, kv)
        den = jnp.einsum("bhqf,bhf->bhq", phi_q, z)[..., None] + 1e-6
        o = num / den
        return (lambda x, *d: x.transpose(*d))(o, 0, 2, 1, 3).reshape(B, S, D) @ wo

    def _B_ref(x, w1, b1, w2, b2):
        h = jnp.einsum("bsd,df->bsf", x, w1) + b1
        h = _gelu(h)
        return jnp.einsum("bsf,fd->bsd", h, w2) + b2

    x = A_x
    xn = _layernorm(x, axis=-1)
    return x + _A_ref(xn, A_wqkv, A_w_phi, A_wo) + _B_ref(xn, B_w1, B_b1, B_w2, B_b2)
```

```python
import numpy as np
import jax
import jax.numpy as jnp
from jax import lax
import jax.experimental.pallas as pl
import jax.experimental.pallas.tpu as pltpu

S, D, H, DH, F = 2048, 448, 16, 28, 1792
HG = 2
G = H // HG
GP = 64
GW = HG * DH
T = 512
NC = S // T
KA = 512
FB = 256
F32, BF16 = jnp.float32, jnp.bfloat16
NT = (((1,), (1,)), ((), ()))


def _dot(a, b):
    return jnp.dot(a, b, preferred_element_type=F32)


def _dot_nt(a, b):
    return lax.dot_general(a, b, NT, preferred_element_type=F32)


def _iota(shape, dim):
    return lax.broadcasted_iota(jnp.int32, shape, dim)


def _group_reduce(x, op):
    r = x[0:8]
    for j in range(1, GW // 8):
        r = op(r, x[8 * j:8 * j + 8])
    sh = 4
    while sh >= HG:
        r = op(r, pltpu.roll(r, sh, 0))
        sh //= 2
    return r


def _tile_rows(r):
    return jnp.concatenate([r] * (GW // 8), axis=0)


def _phi(p):
    mx = _tile_rows(_group_reduce(p, jnp.maximum))
    mn = _tile_rows(_group_reduce(p, jnp.minimum))
    e1 = jnp.exp(p - mx)
    e2 = jnp.exp(mn - p)
    r1 = _tile_rows(1.0 / _group_reduce(e1, jnp.add))
    r2 = _tile_rows(1.0 / _group_reduce(e2, jnp.add))
    return jnp.concatenate([e1 * r1, e2 * r2], axis=0).astype(BF16)


def _kernel(x_hbm, wqkv_hbm, wphi_hbm, wo_hbm, w1_hbm, b1_hbm, w2t_hbm, b2_hbm, o_hbm,
            x_ref, wqkv_ref, wphi_ref, wo_ref, w1_ref, b1_ref, b2_ref,
            xn_ref, aq_ref, akv_ref, w1t_ref, w2t_ref, kv_ref, u_ref, o_ref, sems, osems):
    def chunk(ci):
        return pl.ds(ci * T, T)

    QS = 384
    pairs = [(wphi_hbm, wphi_ref), (wqkv_hbm.at[:, pl.ds(QS, 3 * D - QS)], wqkv_ref.at[:, pl.ds(QS, 3 * D - QS)])]
    pairs += [(x_hbm.at[0, :, chunk(ci)], x_ref.at[:, chunk(ci)]) for ci in range(NC)]
    pairs += [(wo_hbm, wo_ref), (b1_hbm, b1_ref), (b2_hbm, b2_ref), (w1_hbm, w1_ref),
              (w2t_hbm, w2t_ref.at[:, pl.ds(KA, F)]), (wqkv_hbm.at[:, pl.ds(0, QS)], wqkv_ref.at[:, pl.ds(0, QS)])]
    cps = [pltpu.make_async_copy(a, b, sems.at[i]) for i, (a, b) in enumerate(pairs)]
    cp_phi, cp_qkv, cp_x = cps[0], cps[1], cps[2:2 + NC]
    cp_wo, cp_b1, cp_b2, cp_w1, cp_w2, cp_q = cps[2 + NC:]
    for cp in [cp_phi, cp_x[0], cp_qkv, cp_x[1]]:
        cp.start()

    def layernorm_body(ci):
        x = x_ref[:, chunk(ci)].astype(F32)
        m = jnp.mean(x, axis=0, keepdims=True)
        xc = x - m
        var = jnp.mean(xc * xc, axis=0, keepdims=True)
        xn_ref[0:D, chunk(ci)] = (xc * lax.rsqrt(var + 1e-5)).astype(BF16)

    r = _iota((GW, GW), 0)
    c = _iota((GW, GW), 1)
    perm_g = jnp.where(c == (r % HG) * DH + r // HG, 1.0, 0.0).astype(BF16)
    ones_rows = jnp.ones((GP - GW, T), F32)
    one_row = jnp.where(_iota((KA - D, T), 0) == 0, 1.0, 0.0).astype(BF16)
    u_ref[D:KA, :] = one_row
    for ci in range(NC):
        xn_ref[D:KA, chunk(ci)] = one_row
    sel = jnp.where(_iota((GW, DH), 1) == _iota((GW, DH), 0) // HG, 1.0, 0.0).astype(BF16)
    r = _iota((GW, 128), 0)
    tgt = (r % DH) * H + r // DH
    tgt = jnp.concatenate([tgt] * 4, axis=1)[:, :D] - _iota((GW, D), 1)
    stack_sel = [jnp.where(tgt == -HG * g, 1.0, 0.0).astype(BF16) for g in range(G)]
    own = _iota((GW, GW), 1) // DH == _iota((GW, GW), 0) % HG

    cp_phi.wait()
    stack = wphi_ref[...].reshape(D, DH)
    phis = []
    for g in range(G):
        st = _dot(stack_sel[g], stack).astype(BF16)
        phis.append(jnp.where(own, _dot_nt(sel, st), 0.0).astype(BF16))
    cp_x[0].wait()
    layernorm_body(0)
    cp_qkv.wait()
    for cp in [cp_q, cp_x[2], cp_b1, cp_w1]:
        cp.start()

    def fold(mats, col0):
        parts = [_dot_nt(mats[g], wqkv_ref[:, col0 + GW * g:col0 + GW * (g + 1)]) for g in range(G)]
        return jnp.concatenate(parts, axis=0).astype(BF16)

    akv_ref[0:D, :] = fold(phis, D)
    akv_ref[D:2 * D, :] = fold([perm_g] * G, 2 * D)

    kv = [jnp.zeros((GP, 2 * GW), F32) for _ in range(G)]
    for ci in range(NC):
        if ci + 1 < NC:
            cp_x[ci + 1].wait()
        if ci == 2:
            cp_b1.wait()
            cp_w1.wait()
            cp_w2.start()
        pkv = _dot(akv_ref[...], xn_ref[0:D, chunk(ci)])
        if ci + 1 < NC:
            layernorm_body(ci + 1)
        for g in range(G):
            vt = jnp.concatenate([pkv[D + GW * g:D + GW * (g + 1)], ones_rows], axis=0).astype(BF16)
            kv[g] = kv[g] + _dot_nt(vt, _phi(pkv[GW * g:GW * (g + 1)]))
            if ci in (2, 3):
                for j in range(F // 128):
                    if j == G * (ci - 2) + g:
                        cols = pl.ds(128 * j, 128)
                        w1t_ref[cols, 0:D] = w1_ref[:, cols].T
        if ci == 0:
            cp_q.wait()
            for cp in [cp_x[3], cp_wo, cp_b2]:
                cp.start()
            aq_ref[...] = fold(phis, 0)
        if ci == 2:
            b1 = b1_ref[...].astype(F32).reshape(1, F)
            first = _iota((8, F), 0) == 0
            b1t = jnp.concatenate([jnp.where(first, b1, 0.0), jnp.zeros((KA - D - 8, F), F32)], axis=0)
            w1t_ref[:, D:KA] = b1t.T.astype(BF16)
        if ci == 3:
            cp_wo.wait()
            cp_b2.wait()
            wo = wo_ref[...].astype(F32)
            wop = jnp.concatenate([_dot(perm_g, wo[GW * g:GW * (g + 1)].astype(BF16)) for g in range(G)], axis=0)
            w2t_ref[:, 0:D] = wop.T.astype(BF16)
            b2 = b2_ref[...].astype(F32).reshape(1, D)
            first = _iota((8, D), 0) == 0
            b2t = jnp.concatenate([jnp.where(first, b2, 0.0), jnp.zeros((KA - D - 8, D), F32)], axis=0)
            w2t_ref[:, D:KA] = b2t.T.astype(BF16)
    same_head = _iota((GP, 2 * GW), 0) % HG == _iota((GP, 2 * GW), 1) % HG
    for g in range(G):
        kv_ref[g] = jnp.where(same_head, kv[g], 0.0).astype(BF16)

    outs = []
    for ci in range(NC):
        xn = xn_ref[:, chunk(ci)]
        pq = _dot(aq_ref[...], xn[0:D])
        os_ = []
        for j in range(max(F // FB, G)):
            if j < G:
                nd = _dot(kv_ref[j], _phi(pq[GW * j:GW * (j + 1)]))
                os_.append(nd[0:GW] * _tile_rows(1.0 / (nd[GW:GW + 8] + 1e-6)))
                if j == G - 1:
                    u_ref[0:D, :] = jnp.concatenate(os_, axis=0).astype(BF16)
            if j >= F // FB:
                continue
            h = _dot(w1t_ref[pl.ds(FB * j, FB), :], xn)
            t = jnp.tanh(h * (0.7978845608028654 + 0.035677408136300125 * (h * h)))
            u_ref[pl.ds(KA + FB * j, FB), :] = (0.5 * h * (1.0 + t)).astype(BF16)
        if ci == 0:
            cp_w2.wait()
        y = _dot(w2t_ref[...], u_ref[...])
        o_ref[:, chunk(ci)] = (x_ref[:, chunk(ci)].astype(F32) + y).astype(o_ref.dtype)
        cp = pltpu.make_async_copy(o_ref.at[:, chunk(ci)], o_hbm.at[0, :, chunk(ci)], osems.at[ci])
        cp.start()
        outs.append(cp)
    for cp in outs:
        cp.wait()


@jax.jit
def pallas_parallel_sum__linear_kernel_hedgehog__dense_activation_gelu__prompt_kernel(
    A_x, A_wqkv, A_w_phi, A_wo, B_x, B_w1, B_b1, B_w2, B_b2,
):
    del B_x
    hbm = pl.BlockSpec(memory_space=pl.ANY)
    out_t = pl.pallas_call(
        _kernel,
        in_specs=[hbm] * 8,
        out_specs=hbm,
        out_shape=jax.ShapeDtypeStruct((1, D, S), A_x.dtype),
        scratch_shapes=[
            pltpu.VMEM((D, S), BF16),
            pltpu.VMEM((D, 3 * D), BF16),
            pltpu.VMEM((DH, H, DH), BF16),
            pltpu.VMEM((D, D), BF16),
            pltpu.VMEM((D, F), BF16),
            pltpu.VMEM((F,), BF16),
            pltpu.VMEM((D,), BF16),
            pltpu.VMEM((KA, S), BF16),
            pltpu.VMEM((D, D), BF16),
            pltpu.VMEM((2 * D, D), BF16),
            pltpu.VMEM((F, KA), BF16),
            pltpu.VMEM((D, KA + F), BF16),
            pltpu.VMEM((G, GP, 2 * GW), BF16),
            pltpu.VMEM((KA + F, T), BF16),
            pltpu.VMEM((D, S), A_x.dtype),
            pltpu.SemaphoreType.DMA((8 + NC,)),
            pltpu.SemaphoreType.DMA((NC,)),
        ],
        compiler_params=pltpu.CompilerParams(vmem_limit_bytes=100 * 1024 * 1024),
    )(A_x.transpose(0, 2, 1), A_wqkv, A_w_phi.transpose(1, 0, 2), A_wo, B_w1, B_b1, B_w2.T, B_b2)
    return out_t.transpose(0, 2, 1)
```
